```python
import os as _os
_os.environ.setdefault("JAX_PLATFORMS", "cpu")
import jax
import jax.numpy as jnp

def _softmax(x, axis=-1):
    return jax.nn.softmax(x, axis=axis)
def _gelu(x):
    return jax.nn.gelu(x, approximate=True)
def _silu(x):
    return jax.nn.silu(x)
def _sigmoid(x):
    return jax.nn.sigmoid(x)
def _layernorm(x, axis=-1, eps=1e-5):
    m = jnp.mean(x, axis=axis, keepdims=True)
    v = jnp.var(x, axis=axis, keepdims=True)
    return (x - m) / jnp.sqrt(v + eps)
def _scatter_add(tgt, idx, src, axis=0):
    return tgt.at[idx].add(src)
def _segment_sum(src, seg, n):
    return jax.ops.segment_sum(src, seg, n)
class _Rng:
    def __init__(self, key):
        self._k = key
    def _next(self):
        self._k, sub = jax.random.split(self._k)
        return sub
    def normal(self, shape):
        return jax.random.normal(self._next(), shape, dtype=jnp.bfloat16)
    def randint(self, lo, hi, shape):
        return jax.random.randint(self._next(), shape, lo, hi, dtype=jnp.int32)
    def uniform(self, shape, lo=0.0, hi=1.0):
        return jax.random.uniform(self._next(), shape, jnp.bfloat16, lo, hi)
    def permutation(self, n):
        return jax.random.permutation(self._next(), n)


kernel_name = 'sequential_preLN__softmax_full_mha__dense_activation_gelu__prompt'

def setup_inputs():
    _rng = _Rng(jax.random.key(int.from_bytes(__import__("os").urandom(4), "little")))
    _w = (lambda a: (lambda t: t.astype(jnp.bfloat16) if jnp.issubdtype(t.dtype, jnp.floating) else t)(jnp.asarray(a)))
    def _A_setup():
        B, S, D = 1, 2048, 640
        return {
            "x": _w((lambda *s: _rng.normal(s) * 0.05)(B, S, D)),
            "wqkv": _w((lambda *s: _rng.normal(s) * 0.05)(D, 3 * D)),
            "wo": _w((lambda *s: _rng.normal(s) * 0.05)(D, D)),
        }
    _A_in = _A_setup()

    def _B_setup():
        B, S, D, F = 1, 2048, 640, 1536
        return {
            "x": _w((lambda *s: _rng.normal(s) * 0.05)(B, S, D)),
            "w1": _w((lambda *s: _rng.normal(s) * 0.4)(D, F) * (D ** -0.5)),
            "b1": _w((lambda *s: _rng.normal(s) * 0.4)(F) * 0.01),
            "w2": _w((lambda *s: _rng.normal(s) * 0.4)(F, D) * (F ** -0.5)),
            "b2": _w((lambda *s: _rng.normal(s) * 0.05)(D) * 0.01),
        }
    _B_in = _B_setup()

    return {
        "A_x": _A_in["x"],
        "A_wqkv": _A_in["wqkv"],
        "A_wo": _A_in["wo"],
        "B_x": _B_in["x"],
        "B_w1": _B_in["w1"],
        "B_b1": _B_in["b1"],
        "B_w2": _B_in["w2"],
        "B_b2": _B_in["b2"],
    }

def reference(A_x, A_wqkv, A_wo, B_x, B_w1, B_b1, B_w2, B_b2):
    def _A_ref(x, wqkv, wo):
        B, S, D = x.shape
        H = 32; Dh = D // H
        qkv = (lambda x, *d: x.transpose(*d))((x @ wqkv).reshape(B, S, 3, H, Dh), 2, 0, 3, 1, 4)
        q, k, v = qkv[0], qkv[1], qkv[2]
        scale = Dh ** -0.5
        scores = jnp.einsum("bhqd,bhkd->bhqk", q, k) * scale
        p = _softmax(scores, axis=-1)
        o = jnp.einsum("bhqk,bhkd->bhqd", p, v)
        return (lambda x, *d: x.transpose(*d))(o, 0, 2, 1, 3).reshape(B, S, D) @ wo

    def _B_ref(x, w1, b1, w2, b2):
        h = jnp.einsum("bsd,df->bsf", x, w1) + b1
        h = _gelu(h)
        return jnp.einsum("bsf,fd->bsd", h, w2) + b2

    x = A_x
    h = x + _A_ref(_layernorm(x, axis=-1), A_wqkv, A_wo)
    h2 = h + _B_ref(_layernorm(h, axis=-1), B_w1, B_b1, B_w2, B_b2)
    return h2
```

```python
import math

import jax
import jax.numpy as jnp
from jax import lax
import jax.experimental.pallas as pl
import jax.experimental.pallas.tpu as pltpu

S, D, F, H = 2048, 640, 1536, 32
DH = D // H
HPT = 6
NT = 6
RC = 512
NC = S // RC
TQ = 128
NQ = S // TQ
CH = 128
G = 4
UN = 4
MV = 32
EPS = 1e-5
_NT = (((1,), (1,)), ((), ()))
f32, bf16 = jnp.float32, jnp.bfloat16


def _ln(x):
    xc = x - jnp.mean(x, axis=-1, keepdims=True)
    v = jnp.mean(xc * xc, axis=-1, keepdims=True)
    return xc * lax.rsqrt(v + EPS)


def _body(x_hbm, wqkv_hbm, wo_hbm, w1_hbm, b1_ref, w2_hbm, b2_ref, out_hbm,
          x_v, wqkv_v, wo_v, w1_v, w2_v, q_v, k_v, vt_v, ot_v, s0_v, s1_v,
          out_v, xsem, wsem, osem):
    def rows(c):
        return pl.ds(pl.multiple_of(c * RC, RC), RC)

    def x_copy(c):
        return pltpu.make_async_copy(x_hbm.at[rows(c)], x_v.at[rows(c)], xsem.at[c])

    def o_copy(c):
        return pltpu.make_async_copy(out_v.at[rows(c)], out_hbm.at[rows(c)], osem.at[c])

    w_copies = [pltpu.make_async_copy(s, d, wsem.at[i]) for i, (s, d) in enumerate(
        [(wqkv_hbm, wqkv_v), (wo_hbm, wo_v), (w1_hbm, w1_v), (w2_hbm, w2_v)])]
    x_copy(0).start()
    w_copies[0].start()
    for c in range(1, NC):
        x_copy(c).start()
    for cp in w_copies[1:]:
        cp.start()
    w_copies[0].wait()

    qscale = DH ** -0.5 * math.log2(math.e)

    def proj(c, carry):
        x_copy(c).wait()
        xn = _ln(x_v[rows(c), :].astype(f32)).astype(bf16)
        qkv = jnp.dot(xn, wqkv_v[...], preferred_element_type=f32)
        for t in range(NT):
            a = t * HPT * DH
            q_v[t, rows(c), :] = (qkv[:, a:a + 128] * qscale).astype(bf16)
            k_v[t, rows(c), :] = qkv[:, D + a:D + a + 128].astype(bf16)
        vt = qkv[:, 2 * D:].T
        tail = (lax.broadcasted_iota(jnp.int32, (MV - DH, RC), 0) == 0).astype(f32)
        for h in range(H):
            blk = jnp.concatenate([vt[h * DH:(h + 1) * DH], tail], axis=0)
            vt_v[h, :, rows(c)] = blk.astype(bf16)
        return carry

    lax.fori_loop(0, NC, proj, 0)

    s_bufs = (s0_v, s1_v)
    lane = lax.broadcasted_iota(jnp.int32, (TQ, 128), 1)

    def get_q(h, j):
        t = h // HPT
        lo = (h - t * HPT) * DH
        q = q_v[t, pl.ds(pl.multiple_of(j * TQ, TQ), TQ), :]
        return t, jnp.where((lane >= lo) & (lane < lo + DH), q, jnp.zeros_like(q))

    def qk_chunk(t, c, buf, q):
        s = lax.dot_general(k_v[t, pl.ds(c * CH, CH), :], q, _NT,
                            preferred_element_type=f32)
        buf[pl.ds(c * CH, CH), :] = s
        return jnp.max(s.reshape(CH // 8, 8, TQ), axis=0)

    def pv_chunk(h, c, buf, m, acc):
        p = jnp.exp2(buf[pl.ds(c * CH, CH), :] - m).astype(bf16)
        return acc + jnp.dot(vt_v[h, :, pl.ds(c * CH, CH)], p,
                             preferred_element_type=f32)

    def step(u, m8, slot):
        h, j = u // NQ, u % NQ
        un = jnp.minimum(u + 1, H * NQ - 1)
        tn, qn = get_q(un // NQ, un % NQ)
        m = jnp.max(m8, axis=0, keepdims=True)
        acc = jnp.zeros((MV, TQ), f32)
        mn = None
        for g in range(S // CH // G):
            for c in range(g * G, g * G + G):
                mm = qk_chunk(tn, c, s_bufs[1 - slot], qn)
                mn = mm if mn is None else jnp.maximum(mn, mm)
            for c in range(g * G, g * G + G):
                acc = pv_chunk(h, c, s_bufs[slot], m, acc)
        o = acc[:24] * (1.0 / acc[DH:DH + 1])
        ot_v[h, :, pl.ds(pl.multiple_of(j * TQ, TQ), TQ)] = o
        return mn

    t0, q0 = get_q(0, 0)
    m0 = None
    for c in range(S // CH):
        mm = qk_chunk(t0, c, s_bufs[0], q0)
        m0 = mm if m0 is None else jnp.maximum(m0, mm)

    def attn(i, m8):
        for r in range(UN):
            m8 = step(UN * i + r, m8, r % 2)
        return m8

    lax.fori_loop(0, H * NQ // UN, attn, m0)

    for cp in w_copies[1:]:
        cp.wait()

    def ffn(c, carry):
        ot = jnp.concatenate([ot_v[h, :DH, rows(c)] for h in range(H)], axis=0)
        o = ot.T.astype(bf16)
        h1 = x_v[rows(c), :].astype(f32) + jnp.dot(o, wo_v[...], preferred_element_type=f32)
        a = jnp.dot(_ln(h1).astype(bf16), w1_v[...], preferred_element_type=f32)
        a = jax.nn.gelu(a + b1_ref[...].astype(f32), approximate=True)
        y = jnp.dot(a.astype(bf16), w2_v[...], preferred_element_type=f32)
        out_v[rows(c), :] = (h1 + y + b2_ref[...].astype(f32)).astype(bf16)
        o_copy(c).start()
        return carry

    lax.fori_loop(0, NC, ffn, 0)
    for c in range(NC):
        o_copy(c).wait()


@jax.jit
def pallas_sequential_preLN__softmax_full_mha__dense_activation_gelu__prompt_kernel(
    A_x: jax.Array,
    A_wqkv: jax.Array,
    A_wo: jax.Array,
    B_x: jax.Array,
    B_w1: jax.Array,
    B_b1: jax.Array,
    B_w2: jax.Array,
    B_b2: jax.Array,
):
    hbm = pl.BlockSpec(memory_space=pl.ANY)
    vmem = pl.BlockSpec(memory_space=pltpu.VMEM)
    out = pl.pallas_call(
        _body,
        out_shape=jax.ShapeDtypeStruct((S, D), bf16),
        in_specs=[hbm, hbm, hbm, hbm, vmem, hbm, vmem],
        out_specs=hbm,
        scratch_shapes=[
            pltpu.VMEM((S, D), bf16),
            pltpu.VMEM((D, 3 * D), bf16),
            pltpu.VMEM((D, D), bf16),
            pltpu.VMEM((D, F), bf16),
            pltpu.VMEM((F, D), bf16),
            pltpu.VMEM((NT, S, 128), bf16),
            pltpu.VMEM((NT, S, 128), bf16),
            pltpu.VMEM((H, MV, S), bf16),
            pltpu.VMEM((H, 24, S), f32),
            pltpu.VMEM((S, TQ), f32),
            pltpu.VMEM((S, TQ), f32),
            pltpu.VMEM((S, D), bf16),
            pltpu.SemaphoreType.DMA((NC,)),
            pltpu.SemaphoreType.DMA((4,)),
            pltpu.SemaphoreType.DMA((NC,)),
        ],
        compiler_params=pltpu.CompilerParams(vmem_limit_bytes=100 * 1024 * 1024),
        name="block",
    )(A_x.reshape(S, D), A_wqkv, A_wo, B_w1, B_b1.reshape(1, F), B_w2, B_b2.reshape(1, D))
    return out.reshape(A_x.shape)
```

```python
import math

import jax
import jax.numpy as jnp
from jax import lax
import jax.experimental.pallas as pl
import jax.experimental.pallas.tpu as pltpu

S, D, F, H = 2048, 640, 1536, 32
DH = D // H
RC = 512
NC = S // RC
TQ = 128
NQ = S // TQ
CH = 128
G = 4
UN = 16
MV = 32
LAG = 2
EPS = 1e-5
f32, bf16 = jnp.float32, jnp.bfloat16


def _ln(x):
    xc = x - jnp.mean(x, axis=-1, keepdims=True)
    v = jnp.mean(xc * xc, axis=-1, keepdims=True)
    return xc * lax.rsqrt(v + EPS)


def _body(x_hbm, wqkv_hbm, wo_hbm, w1_hbm, b1_ref, w2_hbm, b2_ref, out_hbm,
          x_v, wqkv_v, wo_v, w1_v, w2_v, q_v, k_v, vt_v, ot_v, s0_v, s1_v, s2_v, s3_v,
          out_v, xsem, wsem, osem):
    def rows(c):
        return pl.ds(pl.multiple_of(c * RC, RC), RC)

    def x_copy(c):
        return pltpu.make_async_copy(x_hbm.at[rows(c)], x_v.at[rows(c)], xsem.at[c])

    def o_copy(c):
        return pltpu.make_async_copy(out_v.at[rows(c)], out_hbm.at[rows(c)], osem.at[c])

    w_copies = [pltpu.make_async_copy(s, d, wsem.at[i]) for i, (s, d) in enumerate(
        [(wqkv_hbm, wqkv_v), (wo_hbm, wo_v), (w1_hbm, w1_v), (w2_hbm, w2_v)])]
    x_copy(0).start()
    w_copies[0].start()
    for c in range(1, NC):
        x_copy(c).start()
    for cp in w_copies[1:]:
        cp.start()
    w_copies[0].wait()

    qscale = DH ** -0.5 * math.log2(math.e)

    def proj(c, carry):
        x_copy(c).wait()
        xn = _ln(x_v[rows(c), :].astype(f32)).astype(bf16)
        qkv = jnp.dot(xn, wqkv_v[...], preferred_element_type=f32)
        qt = qkv[:, :D].T * qscale
        vt = qkv[:, 2 * D:].T
        zeros = jnp.zeros((MV - DH, RC), f32)
        tail = (lax.broadcasted_iota(jnp.int32, (MV - DH, RC), 0) == 0).astype(f32)
        for h in range(H):
            a = h * DH
            k_v[h, rows(c), :] = qkv[:, D + a:D + a + MV].astype(bf16)
            q_v[h, :, rows(c)] = jnp.concatenate([qt[a:a + DH], zeros], 0).astype(bf16)
            vt_v[h, :, rows(c)] = jnp.concatenate([vt[a:a + DH], tail], 0).astype(bf16)
        return carry

    lax.fori_loop(0, NC, proj, 0)

    s_bufs = (s0_v, s1_v, s2_v, s3_v)

    def qk_chunk(h, j, c, buf):
        q = q_v[h, :, pl.ds(pl.multiple_of(j * TQ, TQ), TQ)]
        s = jnp.dot(k_v[h, pl.ds(c * CH, CH), :], q, preferred_element_type=f32)
        buf[pl.ds(c * CH, CH), :] = s
        return jnp.max(s.reshape(CH // 8, 8, TQ), axis=0)

    def pv_chunk(h, c, buf, m, acc):
        p = jnp.exp2(buf[pl.ds(c * CH, CH), :] - m).astype(bf16)
        return acc + jnp.dot(vt_v[h, :, pl.ds(c * CH, CH)], p,
                             preferred_element_type=f32)

    def step(u, m8, dep, slot):
        h, j = u // NQ, u % NQ
        un = jnp.minimum(u + 2, H * NQ - 1)
        m = jnp.max(m8, axis=0, keepdims=True)
        acc = jnp.zeros((MV, TQ), f32)
        mn = None
        deps = [m8, m8, dep]
        for g in range(S // CH // G):
            mg = jnp.maximum(m, jnp.minimum(m, deps[-LAG][:1]))
            for c in range(g * G, g * G + G):
                mm = qk_chunk(un // NQ, un % NQ, c, s_bufs[(slot + 2) % 4])
                mn = mm if mn is None else jnp.maximum(mn, mm)
            for c in range(g * G, g * G + G):
                acc = pv_chunk(h, c, s_bufs[slot], mg, acc)
            deps.append(mn)
        o = acc[:24] * (1.0 / acc[DH:DH + 1])
        ot_v[h, :, pl.ds(pl.multiple_of(j * TQ, TQ), TQ)] = o
        return mn

    def fill(u):
        m8 = None
        for c in range(S // CH):
            mm = qk_chunk(0, u, c, s_bufs[u])
            m8 = mm if m8 is None else jnp.maximum(m8, mm)
        return m8

    def attn(i, ms):
        for r in range(UN):
            ms = (ms[1], step(UN * i + r, ms[0], ms[1], r % 4))
        return ms

    lax.fori_loop(0, H * NQ // UN, attn, (fill(0), fill(1)))

    for cp in w_copies[1:]:
        cp.wait()

    def ffn(c, carry):
        ot = jnp.concatenate([ot_v[h, :DH, rows(c)] for h in range(H)], axis=0)
        o = ot.T.astype(bf16)
        h1 = x_v[rows(c), :].astype(f32) + jnp.dot(o, wo_v[...], preferred_element_type=f32)
        a = jnp.dot(_ln(h1).astype(bf16), w1_v[...], preferred_element_type=f32)
        a = jax.nn.gelu(a + b1_ref[...].astype(f32).reshape(1, F), approximate=True)
        y = jnp.dot(a.astype(bf16), w2_v[...], preferred_element_type=f32)
        out_v[rows(c), :] = (h1 + y + b2_ref[...].astype(f32).reshape(1, D)).astype(bf16)
        o_copy(c).start()
        return carry

    lax.fori_loop(0, NC, ffn, 0)
    for c in range(NC):
        o_copy(c).wait()


@jax.jit
def pallas_sequential_preLN__softmax_full_mha__dense_activation_gelu__prompt_kernel(
    A_x: jax.Array,
    A_wqkv: jax.Array,
    A_wo: jax.Array,
    B_x: jax.Array,
    B_w1: jax.Array,
    B_b1: jax.Array,
    B_w2: jax.Array,
    B_b2: jax.Array,
):
    hbm = pl.BlockSpec(memory_space=pl.ANY)
    vmem = pl.BlockSpec(memory_space=pltpu.VMEM)
    out = pl.pallas_call(
        _body,
        out_shape=jax.ShapeDtypeStruct((S, D), bf16),
        in_specs=[hbm, hbm, hbm, hbm, vmem, hbm, vmem],
        out_specs=hbm,
        scratch_shapes=[
            pltpu.VMEM((S, D), bf16),
            pltpu.VMEM((D, 3 * D), bf16),
            pltpu.VMEM((D, D), bf16),
            pltpu.VMEM((D, F), bf16),
            pltpu.VMEM((F, D), bf16),
            pltpu.VMEM((H, MV, S), bf16),
            pltpu.VMEM((H, S, MV), bf16),
            pltpu.VMEM((H, MV, S), bf16),
            pltpu.VMEM((H, 24, S), f32),
            pltpu.VMEM((S, TQ), f32),
            pltpu.VMEM((S, TQ), f32),
            pltpu.VMEM((S, TQ), f32),
            pltpu.VMEM((S, TQ), f32),
            pltpu.VMEM((S, D), bf16),
            pltpu.SemaphoreType.DMA((NC,)),
            pltpu.SemaphoreType.DMA((4,)),
            pltpu.SemaphoreType.DMA((NC,)),
        ],
        compiler_params=pltpu.CompilerParams(vmem_limit_bytes=100 * 1024 * 1024),
        name="block",
    )(A_x.reshape(S, D), A_wqkv, A_wo, B_w1, B_b1, B_w2, B_b2)
    return out.reshape(A_x.shape)
```
